```python
import os as _os
_os.environ.setdefault("JAX_PLATFORMS", "cpu")
import jax
import jax.numpy as jnp

def _softmax(x, axis=-1):
    return jax.nn.softmax(x, axis=axis)
def _gelu(x):
    return jax.nn.gelu(x, approximate=True)
def _silu(x):
    return jax.nn.silu(x)
def _sigmoid(x):
    return jax.nn.sigmoid(x)
def _layernorm(x, axis=-1, eps=1e-5):
    m = jnp.mean(x, axis=axis, keepdims=True)
    v = jnp.var(x, axis=axis, keepdims=True)
    return (x - m) / jnp.sqrt(v + eps)
def _scatter_add(tgt, idx, src, axis=0):
    return tgt.at[idx].add(src)
def _segment_sum(src, seg, n):
    return jax.ops.segment_sum(src, seg, n)
class _Rng:
    def __init__(self, key):
        self._k = key
    def _next(self):
        self._k, sub = jax.random.split(self._k)
        return sub
    def normal(self, shape):
        return jax.random.normal(self._next(), shape, dtype=jnp.bfloat16)
    def randint(self, lo, hi, shape):
        return jax.random.randint(self._next(), shape, lo, hi, dtype=jnp.int32)
    def uniform(self, shape, lo=0.0, hi=1.0):
        return jax.random.uniform(self._next(), shape, jnp.bfloat16, lo, hi)
    def permutation(self, n):
        return jax.random.permutation(self._next(), n)


kernel_name = 'standalone__sliding_local_fixed_window__prompt'

def setup_inputs():
    _rng = _Rng(jax.random.key(int.from_bytes(__import__("os").urandom(4), "little")))
    _w = (lambda a: (lambda t: t.astype(jnp.bfloat16) if jnp.issubdtype(t.dtype, jnp.floating) else t)(jnp.asarray(a)))
    B, H, S, D = 1, 32, 2048, 128
    return {
        "q": _w((lambda *s: _rng.normal(s) * 0.4)(B, H, S, D)),
        "k": _w((lambda *s: _rng.normal(s) * 0.4)(B, H, S, D)),
        "v": _w((lambda *s: _rng.normal(s) * 0.05)(B, H, S, D)),
    }

def reference(q, k, v):
    B, H, S, D = q.shape
    w = 32
    pos = jnp.arange(S)
    rel = pos[:, None] - pos[None, :]
    mask = (rel >= 0) & (rel < w)
    scores = jnp.einsum("bhqd,bhkd->bhqk", q, k) * (D ** -0.5)
    scores = jnp.where(mask[None, None], scores, (lambda x, dt: x.astype(dt))(jnp.array(-1e9), q.dtype))
    p = _softmax(scores, axis=-1)
    return jnp.einsum("bhqk,bhkd->bhqd", p, v)
```

```python
import jax
import jax.numpy as jnp
from jax import lax
import jax.experimental.pallas as pl
import jax.experimental.pallas.tpu as pltpu

_WINDOW = 32
_MASKED_SCORE = -999292928.0
_KEYS = 128
_ROWS = _KEYS - _WINDOW
_WRITE_ROWS = 32
_HEAD_UNROLL = 16
_LOG2E = 1.4426950408889634
_NT = (((1,), (1,)), ((), ()))


@jax.jit
def pallas_standalone__sliding_local_fixed_window__prompt_kernel(
    q: jax.Array,
    k: jax.Array,
    v: jax.Array,
):
    B, H, S, D = q.shape
    G = B * H
    assert (S - _KEYS) % _ROWS == 0 and S % _KEYS == 0 and G % _HEAD_UNROLL == 0
    last = (S - _KEYS) // _ROWS
    assert last >= 3
    scale = D ** -0.5
    fill = _MASKED_SCORE / scale
    to_exp2 = scale * _LOG2E

    def kernel_function(q_hbm, k_hbm, v_hbm, o_hbm, q_buf, k_buf, v_buf, o_buf, low_ref, sems):
        def band_start(i):
            r0 = _WINDOW + _ROWS * i
            return r0 if isinstance(r0, int) else pl.multiple_of(r0, _WINDOW)

        def read(src, dst, r0, rows, slot, heads=slice(None)):
            return pltpu.make_async_copy(
                src.at[heads, pl.ds(r0, rows)], dst.at[heads, pl.ds(r0, rows)], sems.at[slot])

        def read_band(r0, rows, slot):
            return [read(src, dst, r0, rows, slot)
                    for src, dst in ((q_hbm, q_buf), (k_hbm, k_buf), (v_hbm, v_buf))]

        head_slot, tail_slot = last % 2, (last + 1) % 2

        def read_last_head():
            r0 = band_start(last)
            return [read(q_hbm, q_buf, r0, _ROWS, head_slot),
                    read(k_hbm, k_buf, r0, _ROWS, head_slot),
                    read(v_hbm, v_buf, r0, _ROWS, head_slot, pl.ds(0, G // 2))]

        def read_last_tail():
            return read(v_hbm, v_buf, band_start(last), _ROWS, tail_slot, pl.ds(G // 2, G // 2))

        def start_writes(lo, hi):
            def body(i, _):
                r0 = pl.multiple_of(i * _WRITE_ROWS, _WRITE_ROWS)
                pltpu.make_async_copy(
                    o_buf.at[:, pl.ds(r0, _WRITE_ROWS)], o_hbm.at[:, pl.ds(r0, _WRITE_ROWS)],
                    sems.at[head_slot]).start()
            lax.fori_loop(lo // _WRITE_ROWS, hi // _WRITE_ROWS, body, None)

        def scores(qt, kt, offset):
            s = lax.dot_general(qt, kt, _NT, preferred_element_type=jnp.float32)
            rel = (lax.broadcasted_iota(jnp.int32, s.shape, 0)
                   - lax.broadcasted_iota(jnp.int32, s.shape, 1) + offset)
            return jnp.where((rel >= 0) & (rel < _WINDOW), s, fill)

        def tile(h, q0, rows, k0):
            s = scores(q_buf[h, pl.ds(q0, rows), :], k_buf[h, pl.ds(k0, _KEYS), :], _KEYS - rows)
            m = jnp.max(s, axis=1, keepdims=True)
            p = jnp.exp2((s - m) * to_exp2)
            l = jnp.sum(p, axis=1, keepdims=True)
            o = jnp.dot(p.astype(v_buf.dtype), v_buf[h, pl.ds(k0, _KEYS), :],
                        preferred_element_type=jnp.float32)
            o_buf[h, pl.ds(q0, rows), :] = (o * (1.0 / l)).astype(o_buf.dtype)
            return m

        def band(q0, rows, k0):
            def body(g, _):
                low = low_ref[pl.ds(0, rows), :]
                for j in range(_HEAD_UNROLL):
                    low = jnp.minimum(low, tile(g * _HEAD_UNROLL + j, q0, rows, k0))
                low_ref[pl.ds(0, rows), :] = low
            lax.fori_loop(0, G // _HEAD_UNROLL, body, None)

        def dense_tile(t, _):
            h = t // (S // _KEYS)
            q0 = pl.multiple_of((t % (S // _KEYS)) * _KEYS, _KEYS)
            qt = q_buf[h, pl.ds(q0, _KEYS), :]

            def step(j, carry):
                m_old, l, acc = carry
                k0 = pl.multiple_of(j * _KEYS, _KEYS)
                s = scores(qt, k_buf[h, pl.ds(k0, _KEYS), :], q0 - k0)
                m = jnp.maximum(m_old, jnp.max(s, axis=1, keepdims=True))
                p = jnp.exp2((s - m) * to_exp2)
                alpha = jnp.exp2((m_old - m) * to_exp2)
                pv = jnp.dot(p.astype(v_buf.dtype), v_buf[h, pl.ds(k0, _KEYS), :],
                             preferred_element_type=jnp.float32)
                return m, alpha * l + jnp.sum(p, axis=1, keepdims=True), alpha * acc + pv

            init = (jnp.full((_KEYS, 1), fill, jnp.float32),
                    jnp.zeros((_KEYS, 1), jnp.float32),
                    jnp.zeros((_KEYS, D), jnp.float32))
            _, l, acc = lax.fori_loop(0, S // _KEYS, step, init)
            o_buf[h, pl.ds(q0, _KEYS), :] = (acc * (1.0 / l)).astype(o_buf.dtype)

        for copy in read_band(0, _KEYS, 0) + read_band(band_start(1), _ROWS, 1):
            copy.start()
        low_ref[...] = jnp.zeros(low_ref.shape, low_ref.dtype)
        for copy in read_band(0, _KEYS, 0):
            copy.wait()
        for copy in read_band(band_start(2), _ROWS, 0):
            copy.start()
        band(0, _KEYS, 0)

        def band_step(i, _):
            slot = i % 2

            @pl.when(i < last)
            def _():
                for copy in read_band(band_start(i), _ROWS, slot):
                    copy.wait()

                @pl.when(i + 2 < last)
                def _():
                    for copy in read_band(band_start(i + 2), _ROWS, slot):
                        copy.start()

                @pl.when(i + 2 == last)
                def _():
                    for copy in read_last_head():
                        copy.start()

                @pl.when(i + 1 == last)
                def _():
                    read_last_tail().start()

            @pl.when(i == last)
            def _():
                for copy in read_last_head():
                    copy.wait()
                start_writes(0, S - _ROWS)
                read_last_tail().wait()

            band(band_start(i), _ROWS, pl.multiple_of(_ROWS * i, _WINDOW))

        lax.fori_loop(1, last + 1, band_step, None)

        start_writes(S - _ROWS, S)
        masked_keys_count = jnp.min(low_ref[...]) < 0.5 * fill
        write_all = pltpu.make_async_copy(o_buf, o_hbm, sems.at[head_slot])
        write_all.wait()

        @pl.when(masked_keys_count)
        def _():
            lax.fori_loop(0, G * (S // _KEYS), dense_tile, None)
            write_all.start()
            write_all.wait()

    flat = (G, S, D)
    hbm = pl.BlockSpec(memory_space=pltpu.HBM)
    resident = pltpu.VMEM(flat, q.dtype)
    out = pl.pallas_call(
        kernel_function,
        in_specs=[hbm, hbm, hbm],
        out_specs=hbm,
        out_shape=jax.ShapeDtypeStruct(flat, q.dtype),
        scratch_shapes=[resident, resident, resident, resident,
                        pltpu.VMEM((_KEYS, 1), jnp.float32),
                        pltpu.SemaphoreType.DMA((2,))],
        compiler_params=pltpu.CompilerParams(vmem_limit_bytes=80 * 1024 * 1024),
    )(q.reshape(flat), k.reshape(flat), v.reshape(flat))
    return out.reshape(q.shape)
```
